```python
import os as _os
_os.environ.setdefault("JAX_PLATFORMS", "cpu")
import jax
import jax.numpy as jnp

def _softmax(x, axis=-1):
    return jax.nn.softmax(x, axis=axis)
def _gelu(x):
    return jax.nn.gelu(x, approximate=True)
def _silu(x):
    return jax.nn.silu(x)
def _sigmoid(x):
    return jax.nn.sigmoid(x)
def _layernorm(x, axis=-1, eps=1e-5):
    m = jnp.mean(x, axis=axis, keepdims=True)
    v = jnp.var(x, axis=axis, keepdims=True)
    return (x - m) / jnp.sqrt(v + eps)
def _scatter_add(tgt, idx, src, axis=0):
    return tgt.at[idx].add(src)
def _segment_sum(src, seg, n):
    return jax.ops.segment_sum(src, seg, n)
class _Rng:
    def __init__(self, key):
        self._k = key
    def _next(self):
        self._k, sub = jax.random.split(self._k)
        return sub
    def normal(self, shape):
        return jax.random.normal(self._next(), shape, dtype=jnp.bfloat16)
    def randint(self, lo, hi, shape):
        return jax.random.randint(self._next(), shape, lo, hi, dtype=jnp.int32)
    def uniform(self, shape, lo=0.0, hi=1.0):
        return jax.random.uniform(self._next(), shape, jnp.bfloat16, lo, hi)
    def permutation(self, n):
        return jax.random.permutation(self._next(), n)


kernel_name = 'standalone__sliding_block_cached__sampling'

def setup_inputs():
    _rng = _Rng(jax.random.key(int.from_bytes(__import__("os").urandom(4), "little")))
    _w = (lambda a: (lambda t: t.astype(jnp.bfloat16) if jnp.issubdtype(t.dtype, jnp.floating) else t)(jnp.asarray(a)))
    B, Sq, D = 8, 4, 640
    Hq, Hkv, Sk, Dh = 32, 32, 4096, 192
    assert Hq % Hkv == 0, (Hq, Hkv)
    return {
        "x": _w((lambda *s: _rng.normal(s) * 0.8)(B, Sq, D)),
        "k_cache": _w((lambda *s: _rng.normal(s) * 0.8)(B, Hkv, Sk, Dh)),
        "v_cache": _w((lambda *s: _rng.normal(s) * 0.05)(B, Hkv, Sk, Dh)),
        "wq": _w((lambda *s: _rng.normal(s) * 0.8)(D, Hq * Dh) * (D ** -0.5)),
        "wo": _w((lambda *s: _rng.normal(s) * 0.05)(Hq * Dh, D) * ((Hq * Dh) ** -0.5)),
    }

def reference(x, k_cache, v_cache, wq, wo):
    B, Sq, D = x.shape
    Hq, Dh = 32, 192
    Hkv, Sk = k_cache.shape[1], k_cache.shape[2]
    W = min(4096, max(256, Sk // 4))
    rep = Hq // Hkv
    q = (lambda x, *d: x.transpose(*d))((x @ wq).reshape(B, Sq, Hq, Dh), 0, 2, 1, 3)
    k = jnp.repeat(k_cache[:, :, Sk - W:, :], rep, axis=1)
    v = jnp.repeat(v_cache[:, :, Sk - W:, :], rep, axis=1)
    scores = jnp.einsum("bhqd,bhkd->bhqk", q, k) * (Dh ** -0.5)
    p = _softmax(scores, axis=-1)
    o = jnp.einsum("bhqk,bhkd->bhqd", p, v)
    return (lambda x, *d: x.transpose(*d))(o, 0, 2, 1, 3).reshape(B, Sq, Hq * Dh) @ wo
```

```python
import jax
import jax.numpy as jnp
import numpy as np
from jax import lax
import jax.experimental.pallas as pl
import jax.experimental.pallas.tpu as pltpu

_HQ = 32
_DH = 192
_DP = 2 * _DH
_STRIPE = 8
_AHEAD = 2
_SLOTS = _AHEAD + 1


def _kv_schedule():
    n, a = _DP // _STRIPE, 4
    order = [(w, hi * a + lo) for lo in range(a) for hi in range(n // a) for w in (0, 1)]
    return tuple((w, s, (t // 2) % 2) for t, (w, s) in enumerate(order))


def _kernel(x_hbm, k_hbm, v_hbm, wq_hbm, wo_hbm, o_hbm,
            xb, kb, vb, wqb, wob, qbd, obd, acc, ob, ksem, vsem, sems,
            *, window, scale):
    B, Sq, D = xb.shape
    Sk = k_hbm.shape[2]
    HP = _HQ // 2
    M = 2 * Sq
    n = HP * B
    sched = _kv_schedule()
    half = len(sched) // 2

    def issue_kv(i, part):
        slot, b, row0 = i % _SLOTS, i % B, (i // B) * _DP
        for w, s, queue in part:
            src, buf, sem = ((k_hbm, kb, ksem), (v_hbm, vb, vsem))[w]
            r0 = pl.multiple_of(row0 + s * _STRIPE, _STRIPE)
            pltpu.make_async_copy(
                src.at[b, pl.ds(r0, _STRIPE), pl.ds(Sk - window, window)],
                buf.at[slot, pl.ds(s * _STRIPE, _STRIPE), :],
                sem.at[slot]).start(priority=queue)

    def issue_wo(hp):
        for t in range(_DP // 16):
            r0 = pl.multiple_of(hp * _DP + ((t % 6) * 4 + t // 6) * 16, 16)
            pltpu.make_async_copy(wo_hbm.at[pl.ds(r0, 16), :], wob.at[pl.ds(r0, 16), :],
                                  sems.at[2]).start(priority=t % 2)

    def wait_all(buf, sem):
        pltpu.make_async_copy(buf, buf, sem).wait()

    pltpu.make_async_copy(x_hbm, xb, sems.at[0]).start()

    def wq_body(j, carry):
        for t in range(48):
            r0 = pl.multiple_of(j * 64 + (t % 8) * 8, 8)
            cols = pl.ds((t // 8) * 1024, 1024)
            pltpu.make_async_copy(wq_hbm.at[pl.ds(r0, 8), cols], wqb.at[pl.ds(r0, 8), cols],
                                  sems.at[1]).start(priority=t % 2)
        return carry
    lax.fori_loop(0, D // 64, wq_body, 0)

    wait_all(xb, sems.at[0])
    for b in range(B):
        xf = xb[b].astype(jnp.float32)
        acc[pl.ds(b * M, Sq), :] = xf
        acc[pl.ds(b * M + Sq, Sq), :] = xf
    xdup = acc[...].astype(jnp.bfloat16)
    acc[...] = jnp.zeros_like(acc)

    row = lax.broadcasted_iota(jnp.int32, (B * M, _DP), 0)
    col = lax.broadcasted_iota(jnp.int32, (B * M, _DP), 1)
    diag = ((row % M) < Sq) == (col < _DH)

    for hp in range(3):
        issue_wo(hp)
    wait_all(wqb, sems.at[1])

    def q_body(hp, carry):
        c0 = pl.multiple_of(hp * _DP, 128)
        q = jnp.dot(xdup, wqb[:, pl.ds(c0, _DP)], preferred_element_type=jnp.float32)
        qbd[hp] = jnp.where(diag, q, 0.0)

        @pl.when(hp + 3 < HP)
        def _():
            issue_wo(hp + 3)
        return carry
    lax.fori_loop(0, HP, q_body, 0)

    def kv_prologue(i, carry):
        issue_kv(i, sched)
        return carry
    lax.fori_loop(0, _AHEAD, kv_prologue, 0)
    wait_all(wob, sems.at[2])

    def body(i, carry):
        hp, b, slot = i // B, i % B, i % _SLOTS
        r = pl.ds(pl.multiple_of(b * M, M), M)
        q2 = qbd[hp, r, :].astype(jnp.bfloat16)
        wait_all(kb.at[slot], ksem.at[slot])
        s = jnp.dot(q2, kb[slot], preferred_element_type=jnp.float32) * scale
        m = jnp.max(s, axis=-1, keepdims=True)
        e = jnp.exp(s - m)
        l = jnp.sum(e, axis=-1, keepdims=True)

        @pl.when(i + _AHEAD < n)
        def _():
            issue_kv(i + _AHEAD, sched[:half])

        wait_all(vb.at[slot], vsem.at[slot])
        o = lax.dot_general(e.astype(jnp.bfloat16), vb[slot], (((1,), (1,)), ((), ())),
                            preferred_element_type=jnp.float32)
        obd[r, :] = o / l

        @pl.when(i + _AHEAD < n)
        def _():
            issue_kv(i + _AHEAD, sched[half:])

        @pl.when(b == B - 1)
        def _():
            o2 = jnp.where(diag, obd[...], 0.0).astype(jnp.bfloat16)
            w = wob[pl.ds(pl.multiple_of(hp * _DP, _DP), _DP), :]
            acc[...] += jnp.dot(o2, w, preferred_element_type=jnp.float32)
        return carry
    lax.fori_loop(0, n, body, 0)

    for b in range(B):
        ob[b] = (acc[pl.ds(b * M, Sq), :] + acc[pl.ds(b * M + Sq, Sq), :]).astype(ob.dtype)
    out_copy = pltpu.make_async_copy(ob, o_hbm, sems.at[0])
    out_copy.start()
    out_copy.wait()


@jax.jit
def pallas_standalone__sliding_block_cached__sampling_kernel(
    x: jax.Array,
    k_cache: jax.Array,
    v_cache: jax.Array,
    wq: jax.Array,
    wo: jax.Array,
):
    B, Sq, D = x.shape
    Hkv, Sk = k_cache.shape[1], k_cache.shape[2]
    assert Hkv == _HQ and 2 * Sq == 8 and k_cache.shape[3] == _DH
    window = min(4096, max(256, Sk // 4))
    scale = float(np.asarray(_DH ** -0.5).astype(x.dtype))

    kt = jnp.swapaxes(k_cache, 2, 3).reshape(B, Hkv * _DH, Sk)
    vt = jnp.swapaxes(v_cache, 2, 3).reshape(B, Hkv * _DH, Sk)

    def kernel(*refs):
        _kernel(*refs, window=window, scale=scale)

    hbm = pl.BlockSpec(memory_space=pltpu.HBM)
    return pl.pallas_call(
        kernel,
        out_shape=jax.ShapeDtypeStruct(x.shape, x.dtype),
        in_specs=[hbm] * 5,
        out_specs=hbm,
        scratch_shapes=[
            pltpu.VMEM(x.shape, x.dtype),
            pltpu.VMEM((_SLOTS, _DP, window), k_cache.dtype),
            pltpu.VMEM((_SLOTS, _DP, window), v_cache.dtype),
            pltpu.VMEM(wq.shape, wq.dtype),
            pltpu.VMEM(wo.shape, wo.dtype),
            pltpu.VMEM((_HQ // 2, B * 2 * Sq, _DP), jnp.float32),
            pltpu.VMEM((B * 2 * Sq, _DP), jnp.float32),
            pltpu.VMEM((B * 2 * Sq, D), jnp.float32),
            pltpu.VMEM(x.shape, x.dtype),
            pltpu.SemaphoreType.DMA((_SLOTS,)),
            pltpu.SemaphoreType.DMA((_SLOTS,)),
            pltpu.SemaphoreType.DMA((3,)),
        ],
        compiler_params=pltpu.CompilerParams(vmem_limit_bytes=64 * 1024 * 1024),
    )(x, kt, vt, wq, wo)
```

```python
import itertools

import jax
import jax.numpy as jnp
import numpy as np
from jax import lax
import jax.experimental.pallas as pl
import jax.experimental.pallas.tpu as pltpu

_HQ = 32
_DH = 192
_DP = 2 * _DH
_ROWS = 8
_WQ_COLS = 1024
_WQ_STRIDE = 4
_WO_ROWS = 16
_WO_STRIDE = 18
_AHEAD = 2
_SLOTS = _AHEAD + 1


def _mixed_radix(digits):
    return [sum(w * i for (w, _), i in zip(digits, idx))
            for idx in itertools.product(*(range(n) for _, n in digits))]


_KV_ORDER = tuple(_mixed_radix(((8, 2), (4, 2), (48, 2), (2, 2), (1, 2), (16, 3))))
_WO_LAST_ORDER = tuple(_mixed_radix(((1, 4), (4, 6))))


def _kernel(x_hbm, k_hbm, v_hbm, wq_hbm, wo_hbm, o_hbm,
            xb, xs, kvb, wqb, wob, qbd, obd, acc, ob, sem, *, window, scale):
    B, Sq, D = xb.shape
    Sk = k_hbm.shape[2]
    HP = _HQ // 2
    M = 2 * Sq
    n = HP * B
    wo_early = (HP - 1) * _DP
    half = len(_KV_ORDER) // 2

    def start_kv(i, order):
        slot, b, row0 = i % _SLOTS, i % B, (i // B) * _DP
        for t, p in enumerate(order):
            which, r = divmod(p * _ROWS, _DP)
            rows = pl.ds(pl.multiple_of(row0 + r, _ROWS), _ROWS)
            pltpu.make_async_copy(
                (k_hbm, v_hbm)[which].at[b, rows, pl.ds(Sk - window, window)],
                kvb.at[slot, which, pl.ds(r, _ROWS), :],
                sem.at[slot]).start(priority=t % 2)

    def start_wo(row0, s, queue):
        rows = pl.ds(row0, _WO_ROWS)
        pltpu.make_async_copy(wo_hbm.at[rows, :], wob.at[rows, :], s).start(priority=queue)

    def wait_filled(buf, s):
        pltpu.make_async_copy(buf, buf, s).wait()

    def diag(rows):
        row = lax.broadcasted_iota(jnp.int32, (rows, _DP), 0)
        col = lax.broadcasted_iota(jnp.int32, (rows, _DP), 1)
        return ((row % M) < Sq) == (col < _DH)

    def project_q(hp):
        cols = pl.ds(pl.multiple_of(hp * _DP, 128), _DP)
        q = jnp.dot(xs[...].astype(wqb.dtype), wqb[:, cols], preferred_element_type=jnp.float32)
        qbd[hp] = jnp.where(diag(B * M), q, 0.0)

    x_copy = pltpu.make_async_copy(x_hbm, xb, sem.at[0])
    x_copy.start()

    def wq_body(j, carry):
        cols = pl.ds(pl.multiple_of((j // _WQ_STRIDE) * _WQ_COLS, _WQ_COLS), _WQ_COLS)
        for t in range(D // (_ROWS * _WQ_STRIDE)):
            r0 = pl.multiple_of((j % _WQ_STRIDE + t * _WQ_STRIDE) * _ROWS, _ROWS)
            pltpu.make_async_copy(wq_hbm.at[pl.ds(r0, _ROWS), cols],
                                  wqb.at[pl.ds(r0, _ROWS), cols],
                                  sem.at[1]).start(priority=t % 2)
        return carry
    lax.fori_loop(0, (_HQ * _DH // _WQ_COLS) * _WQ_STRIDE, wq_body, 0)

    def wo_body(j, carry):
        for t in range(wo_early // (_WO_ROWS * _WO_STRIDE)):
            r0 = pl.multiple_of((j + t * _WO_STRIDE) * _WO_ROWS, _WO_ROWS)
            start_wo(r0, sem.at[2], t % 2)
        return carry
    lax.fori_loop(0, _WO_STRIDE, wo_body, 0)

    x_copy.wait()
    for b in range(B):
        xf = xb[b].astype(jnp.float32)
        xs[pl.ds(b * M, Sq), :] = xf
        xs[pl.ds(b * M + Sq, Sq), :] = xf
    acc[...] = jnp.zeros_like(acc)
    obd[...] = jnp.zeros_like(obd)

    start_kv(0, _KV_ORDER)
    wait_filled(wqb, sem.at[1])
    project_q(0)
    start_kv(1, _KV_ORDER)
    wait_filled(wob.at[pl.ds(0, wo_early)], sem.at[2])

    def body(i, carry):
        hp, b, slot = i // B, i % B, i % _SLOTS
        q2 = qbd[hp, pl.ds(pl.multiple_of(b * M, M), M), :].astype(kvb.dtype)
        wait_filled(kvb.at[slot], sem.at[slot])

        s = jnp.dot(q2, kvb[slot, 0], preferred_element_type=jnp.float32) * scale
        e = jnp.exp(s - jnp.max(s, axis=-1, keepdims=True))
        l = jnp.sum(e, axis=-1, keepdims=True)

        @pl.when(i + _AHEAD < n)
        def _():
            start_kv(i + _AHEAD, _KV_ORDER[:half])

        @pl.when(i + _AHEAD == n)
        def _():
            for t, p in enumerate(_WO_LAST_ORDER):
                start_wo(wo_early + p * _WO_ROWS, sem.at[n % _SLOTS], t % 2)

        o = lax.dot_general(e.astype(kvb.dtype), kvb[slot, 1], (((1,), (1,)), ((), ())),
                            preferred_element_type=jnp.float32) / l
        o = jnp.where(diag(M), o, pltpu.roll(o, Sq, 0))
        rows = pl.ds(pl.multiple_of((b // 2) * M, M), M)
        mine = lax.broadcasted_iota(jnp.int32, (M, _DP), 0) // Sq == b % 2
        obd[rows, :] = jnp.where(mine, o, obd[rows, :])

        @pl.when(i + _AHEAD < n)
        def _():
            start_kv(i + _AHEAD, _KV_ORDER[half:])

        @pl.when(i == n - 1)
        def _():
            wait_filled(wob.at[pl.ds(wo_early, _DP)], sem.at[n % _SLOTS])

        @pl.when(jnp.logical_and(b == B // 2 - 1, hp + 1 < HP))
        def _():
            project_q(hp + 1)

        @pl.when(b == B - 1)
        def _():
            w = wob[pl.ds(pl.multiple_of(hp * _DP, _DP), _DP), :]
            acc[...] += jnp.dot(obd[...].astype(wob.dtype), w, preferred_element_type=jnp.float32)
        return carry
    lax.fori_loop(0, n, body, 0)

    for b in range(B):
        ob[b] = acc[pl.ds(b * Sq, Sq), :].astype(ob.dtype)
    out_copy = pltpu.make_async_copy(ob, o_hbm, sem.at[0])
    out_copy.start()
    out_copy.wait()


@jax.jit
def pallas_standalone__sliding_block_cached__sampling_kernel(
    x: jax.Array,
    k_cache: jax.Array,
    v_cache: jax.Array,
    wq: jax.Array,
    wo: jax.Array,
):
    B, Sq, D = x.shape
    Hkv, Sk = k_cache.shape[1], k_cache.shape[2]
    assert Hkv == _HQ and k_cache.shape[3] == _DH and 2 * Sq == 8 and B % 2 == 0
    assert D % (_ROWS * _WQ_STRIDE) == 0
    window = min(4096, max(256, Sk // 4))
    scale = float(np.asarray(_DH ** -0.5).astype(x.dtype))

    kt = jnp.swapaxes(k_cache, 2, 3).reshape(B, Hkv * _DH, Sk)
    vt = jnp.swapaxes(v_cache, 2, 3).reshape(B, Hkv * _DH, Sk)

    def kernel(*refs):
        _kernel(*refs, window=window, scale=scale)

    hbm = pl.BlockSpec(memory_space=pltpu.HBM)
    return pl.pallas_call(
        kernel,
        out_shape=jax.ShapeDtypeStruct(x.shape, x.dtype),
        in_specs=[hbm] * 5,
        out_specs=hbm,
        scratch_shapes=[
            pltpu.VMEM(x.shape, x.dtype),
            pltpu.VMEM((B * 2 * Sq, D), jnp.float32),
            pltpu.VMEM((_SLOTS, 2, _DP, window), k_cache.dtype),
            pltpu.VMEM(wq.shape, wq.dtype),
            pltpu.VMEM(wo.shape, wo.dtype),
            pltpu.VMEM((_HQ // 2, B * 2 * Sq, _DP), jnp.float32),
            pltpu.VMEM((B * Sq, _DP), jnp.float32),
            pltpu.VMEM((B * Sq, D), jnp.float32),
            pltpu.VMEM(x.shape, x.dtype),
            pltpu.SemaphoreType.DMA((_SLOTS,)),
        ],
        compiler_params=pltpu.CompilerParams(
            vmem_limit_bytes=64 * 1024 * 1024,
            disable_bounds_checks=True,
        ),
    )(x, kt, vt, wq, wo)
```

```python
import itertools

import jax
import jax.numpy as jnp
import numpy as np
from jax import lax
import jax.experimental.pallas as pl
import jax.experimental.pallas.tpu as pltpu

_HQ = 32
_DH = 192
_DP = 2 * _DH
_ROWS = 8
_WQ_COLS = 1024
_WQ_STRIDE = 4
_WO_ROWS = 16
_WO_STRIDE = 26
_AHEAD = 2
_SLOTS = _AHEAD + 1
_LATE = 3


def _mixed_radix(digits):
    return [sum(w * i for (w, _), i in zip(digits, idx))
            for idx in itertools.product(*(range(n) for _, n in digits))]


_KV_ORDER = tuple(_mixed_radix(((8, 2), (4, 2), (2, 2), (48, 2), (1, 2), (16, 3))))
_WO_LATE_ORDER = tuple(_mixed_radix(((1, 4), (4, 6))))


def _kernel(x_hbm, k_hbm, v_hbm, wq_hbm, wo_hbm, o_hbm,
            xb, xs, kvb, wqb, wob, qbd, obd, acc, ob, sem, late_sem, *, window, scale):
    B, Sq, D = xb.shape
    Sk = k_hbm.shape[2]
    HP = _HQ // 2
    M = 2 * Sq
    n = HP * B
    wo_early = (HP - _LATE) * _DP
    half = len(_KV_ORDER) // 2

    def start_kv(i, order):
        slot, b, row0 = i % _SLOTS, i % B, (i // B) * _DP
        for t, p in enumerate(order):
            which, r = divmod(p * _ROWS, _DP)
            rows = pl.ds(pl.multiple_of(row0 + r, _ROWS), _ROWS)
            pltpu.make_async_copy(
                (k_hbm, v_hbm)[which].at[b, rows, pl.ds(Sk - window, window)],
                kvb.at[slot, which, pl.ds(r, _ROWS), :],
                sem.at[slot]).start(priority=t % 2)

    def start_wo(row0, s, queue):
        rows = pl.ds(row0, _WO_ROWS)
        pltpu.make_async_copy(wo_hbm.at[rows, :], wob.at[rows, :], s).start(priority=queue)

    def wait_filled(buf, s):
        pltpu.make_async_copy(buf, buf, s).wait()

    def diag(rows):
        row = lax.broadcasted_iota(jnp.int32, (rows, _DP), 0)
        col = lax.broadcasted_iota(jnp.int32, (rows, _DP), 1)
        return ((row % M) < Sq) == (col < _DH)

    def project_q(hp):
        cols = pl.ds(pl.multiple_of(hp * _DP, 128), _DP)
        q = jnp.dot(xs[...].astype(wqb.dtype), wqb[:, cols], preferred_element_type=jnp.float32)
        qbd[hp] = jnp.where(diag(B * M), q, 0.0)

    def project_out(hp):
        w = wob[pl.ds(pl.multiple_of(hp * _DP, _DP), _DP), :]
        acc[...] += jnp.dot(obd[hp % _LATE].astype(wob.dtype), w,
                            preferred_element_type=jnp.float32)

    x_copy = pltpu.make_async_copy(x_hbm, xb, sem.at[0])
    x_copy.start()

    def wq_body(j, carry):
        cols = pl.ds(pl.multiple_of((j // _WQ_STRIDE) * _WQ_COLS, _WQ_COLS), _WQ_COLS)
        for t in range(D // (_ROWS * _WQ_STRIDE)):
            r0 = pl.multiple_of((j % _WQ_STRIDE + t * _WQ_STRIDE) * _ROWS, _ROWS)
            pltpu.make_async_copy(wq_hbm.at[pl.ds(r0, _ROWS), cols],
                                  wqb.at[pl.ds(r0, _ROWS), cols],
                                  sem.at[1]).start(priority=t % 2)
        return carry
    lax.fori_loop(0, (_HQ * _DH // _WQ_COLS) * _WQ_STRIDE, wq_body, 0)

    def wo_body(j, carry):
        for t in range(wo_early // (_WO_ROWS * _WO_STRIDE)):
            r0 = pl.multiple_of((j + t * _WO_STRIDE) * _WO_ROWS, _WO_ROWS)
            start_wo(r0, sem.at[2], t % 2)
        return carry
    lax.fori_loop(0, _WO_STRIDE, wo_body, 0)

    x_copy.wait()
    for b in range(B):
        xf = xb[b].astype(jnp.float32)
        xs[pl.ds(b * M, Sq), :] = xf
        xs[pl.ds(b * M + Sq, Sq), :] = xf
    acc[...] = jnp.zeros_like(acc)
    obd[...] = jnp.zeros_like(obd)

    start_kv(0, _KV_ORDER)
    wait_filled(wqb, sem.at[1])
    project_q(0)
    start_kv(1, _KV_ORDER)
    wait_filled(wob.at[pl.ds(0, wo_early)], sem.at[2])

    def body(i, carry):
        hp, b, slot = i // B, i % B, i % _SLOTS
        q2 = qbd[hp, pl.ds(pl.multiple_of(b * M, M), M), :].astype(kvb.dtype)
        wait_filled(kvb.at[slot], sem.at[slot])

        s = jnp.dot(q2, kvb[slot, 0], preferred_element_type=jnp.float32) * scale
        e = jnp.exp(s - jnp.max(s, axis=-1, keepdims=True))
        l = jnp.sum(e, axis=-1, keepdims=True)

        @pl.when(i + _AHEAD < n)
        def _():
            start_kv(i + _AHEAD, _KV_ORDER[:half])

        @pl.when(i + _AHEAD == n)
        def _():
            for j in range(_LATE):
                for t, p in enumerate(_WO_LATE_ORDER):
                    start_wo(wo_early + j * _DP + p * _WO_ROWS, late_sem.at[j], t % 2)

        o = lax.dot_general(e.astype(kvb.dtype), kvb[slot, 1], (((1,), (1,)), ((), ())),
                            preferred_element_type=jnp.float32) / l
        o = jnp.where(diag(M), o, pltpu.roll(o, Sq, 0))
        rows = pl.ds(pl.multiple_of((b // 2) * M, M), M)
        mine = lax.broadcasted_iota(jnp.int32, (M, _DP), 0) // Sq == b % 2
        obd[hp % _LATE, rows, :] = jnp.where(mine, o, obd[hp % _LATE, rows, :])

        @pl.when(i + _AHEAD < n)
        def _():
            start_kv(i + _AHEAD, _KV_ORDER[half:])

        @pl.when(jnp.logical_and(b == B // 2 - 1, hp + 1 < HP))
        def _():
            project_q(hp + 1)

        @pl.when(jnp.logical_and(b == B - 1, hp < HP - _LATE))
        def _():
            project_out(hp)
        return carry
    lax.fori_loop(0, n, body, 0)

    for j in range(_LATE):
        wait_filled(wob.at[pl.ds(wo_early + j * _DP, _DP)], late_sem.at[j])
        project_out(HP - _LATE + j)

    for b in range(B):
        ob[b] = acc[pl.ds(b * Sq, Sq), :].astype(ob.dtype)
    out_copy = pltpu.make_async_copy(ob, o_hbm, sem.at[0])
    out_copy.start()
    out_copy.wait()


@jax.jit
def pallas_standalone__sliding_block_cached__sampling_kernel(
    x: jax.Array,
    k_cache: jax.Array,
    v_cache: jax.Array,
    wq: jax.Array,
    wo: jax.Array,
):
    B, Sq, D = x.shape
    Hkv, Sk = k_cache.shape[1], k_cache.shape[2]
    assert Hkv == _HQ and k_cache.shape[3] == _DH and 2 * Sq == 8 and B % 2 == 0
    assert D % (_ROWS * _WQ_STRIDE) == 0 and (_HQ * _DH) % _WQ_COLS == 0
    assert ((_HQ // 2 - _LATE) * _DP) % (_WO_ROWS * _WO_STRIDE) == 0
    window = min(4096, max(256, Sk // 4))
    scale = float(np.asarray(_DH ** -0.5).astype(x.dtype))

    kt = jnp.swapaxes(k_cache, 2, 3).reshape(B, Hkv * _DH, Sk)
    vt = jnp.swapaxes(v_cache, 2, 3).reshape(B, Hkv * _DH, Sk)

    def kernel(*refs):
        _kernel(*refs, window=window, scale=scale)

    hbm = pl.BlockSpec(memory_space=pltpu.HBM)
    return pl.pallas_call(
        kernel,
        out_shape=jax.ShapeDtypeStruct(x.shape, x.dtype),
        in_specs=[hbm] * 5,
        out_specs=hbm,
        scratch_shapes=[
            pltpu.VMEM(x.shape, x.dtype),
            pltpu.VMEM((B * 2 * Sq, D), jnp.float32),
            pltpu.VMEM((_SLOTS, 2, _DP, window), k_cache.dtype),
            pltpu.VMEM(wq.shape, wq.dtype),
            pltpu.VMEM(wo.shape, wo.dtype),
            pltpu.VMEM((_HQ // 2, B * 2 * Sq, _DP), jnp.float32),
            pltpu.VMEM((_LATE, B * Sq, _DP), jnp.float32),
            pltpu.VMEM((B * Sq, D), jnp.float32),
            pltpu.VMEM(x.shape, x.dtype),
            pltpu.SemaphoreType.DMA((_SLOTS,)),
            pltpu.SemaphoreType.DMA((_LATE,)),
        ],
        compiler_params=pltpu.CompilerParams(
            vmem_limit_bytes=64 * 1024 * 1024,
            disable_bounds_checks=True,
        ),
    )(x, kt, vt, wq, wo)
```
